```python
import os as _os
_os.environ.setdefault("JAX_PLATFORMS", "cpu")
import jax
import jax.numpy as jnp

def _softmax(x, axis=-1):
    return jax.nn.softmax(x, axis=axis)
def _gelu(x):
    return jax.nn.gelu(x, approximate=True)
def _silu(x):
    return jax.nn.silu(x)
def _sigmoid(x):
    return jax.nn.sigmoid(x)
def _layernorm(x, axis=-1, eps=1e-5):
    m = jnp.mean(x, axis=axis, keepdims=True)
    v = jnp.var(x, axis=axis, keepdims=True)
    return (x - m) / jnp.sqrt(v + eps)
def _scatter_add(tgt, idx, src, axis=0):
    return tgt.at[idx].add(src)
def _segment_sum(src, seg, n):
    return jax.ops.segment_sum(src, seg, n)
class _Rng:
    def __init__(self, key):
        self._k = key
    def _next(self):
        self._k, sub = jax.random.split(self._k)
        return sub
    def normal(self, shape):
        return jax.random.normal(self._next(), shape, dtype=jnp.bfloat16)
    def randint(self, lo, hi, shape):
        return jax.random.randint(self._next(), shape, lo, hi, dtype=jnp.int32)
    def uniform(self, shape, lo=0.0, hi=1.0):
        return jax.random.uniform(self._next(), shape, jnp.bfloat16, lo, hi)
    def permutation(self, n):
        return jax.random.permutation(self._next(), n)


kernel_name = 'interleave_layers__mha_block__dense_activation_mish__prompt'

def setup_inputs():
    _rng = _Rng(jax.random.key(int.from_bytes(__import__("os").urandom(4), "little")))
    _w = (lambda a: (lambda t: t.astype(jnp.bfloat16) if jnp.issubdtype(t.dtype, jnp.floating) else t)(jnp.asarray(a)))
    def _A_setup():
        B, S, D, H = 1, 2048, 512, 32
        return {
            "x": _w((lambda *s: _rng.normal(s) * 0.05)(B, S, D)),
            "wqkv": _w((lambda *s: _rng.normal(s) * 0.05)(D, 3 * D)),
            "wo": _w((lambda *s: _rng.normal(s) * 0.05)(D, D)),
        }
    _A_in = _A_setup()

    def _B_setup():
        B, S, D, F = 1, 2048, 512, 1792
        return {
            "x": _w((lambda *s: _rng.normal(s) * 0.05)(B, S, D)),
            "w1": _w((lambda *s: _rng.normal(s) * 0.4)(D, F) * (D ** -0.5)),
            "b1": _w((lambda *s: _rng.normal(s) * 0.4)(F)),
            "w2": _w((lambda *s: _rng.normal(s) * 0.4)(F, D) * (F ** -0.5)),
        }
    _B_in = _B_setup()

    return {
        "A_x": _A_in["x"],
        "A_wqkv": _A_in["wqkv"],
        "A_wo": _A_in["wo"],
        "B_x": _B_in["x"],
        "B_w1": _B_in["w1"],
        "B_b1": _B_in["b1"],
        "B_w2": _B_in["w2"],
    }

def reference(A_x, A_wqkv, A_wo, B_x, B_w1, B_b1, B_w2):
    def _A_ref(x, wqkv, wo):
        B, S, D = x.shape
        H = 32
        Dh = D // H
        qkv = (lambda x, *d: x.transpose(*d))((x @ wqkv).reshape(B, S, 3, H, Dh), 2, 0, 3, 1, 4)
        q, k, v = qkv[0], qkv[1], qkv[2]
        scores = jnp.einsum("bhqd,bhkd->bhqk", q, k) * (Dh ** -0.5)
        p = _softmax(scores, axis=-1)
        o = jnp.einsum("bhqk,bhkd->bhqd", p, v)
        return (lambda x, *d: x.transpose(*d))(o, 0, 2, 1, 3).reshape(B, S, D) @ wo

    def _B_ref(x, w1, b1, w2):
        h = jnp.einsum("bsd,df->bsf", x, w1) + b1
        sp = jnp.log1p(jnp.exp(-jnp.abs(h))) + jnp.where(h > 0, h, jnp.zeros_like(h))
        act = h * jnp.tanh(sp)
        return jnp.einsum("bsf,fd->bsd", act, w2)

    x = A_x
    x = x + _A_ref(_layernorm(x, axis=-1), A_wqkv, A_wo)
    x = x + _B_ref(_layernorm(x, axis=-1), B_w1, B_b1, B_w2)
    x = x + _A_ref(_layernorm(x, axis=-1), A_wqkv, A_wo)
    x = x + _B_ref(_layernorm(x, axis=-1), B_w1, B_b1, B_w2)
    return x
```

```python
import functools
import math

import jax
import jax.numpy as jnp
import numpy as np
from jax import lax
import jax.experimental.pallas as pl
import jax.experimental.pallas.tpu as pltpu

S, D, H, DH, F = 2048, 512, 32, 16, 1792
LOG2E = 1.4426950408889634
EPS = 1e-5
BF16, F32, I32 = jnp.bfloat16, jnp.float32, jnp.int32


def _dot(a, b):
    return jnp.dot(a, b, preferred_element_type=F32)


def _dot_nt(a, b):
    return lax.dot_general(a, b, (((1,), (1,)), ((), ())), preferred_element_type=F32)


def _dot_tn(a, b):
    return lax.dot_general(a, b, (((0,), (0,)), ((), ())), preferred_element_type=F32)


def _p32(x):
    return pltpu.bitcast(x, I32)


def _u32(x):
    return pltpu.bitcast(x, BF16)


def _layernorm(x):
    m = jnp.mean(x, axis=-1, keepdims=True)
    xc = x - m
    v = jnp.mean(xc * xc, axis=-1, keepdims=True)
    return xc * lax.rsqrt(v + EPS)


def _mish(h):
    sp = jnp.log1p(jnp.exp(-jnp.abs(h))) + jnp.maximum(h, 0.0)
    return h * jnp.tanh(sp)


def make(TM=512, FC=256, NQ=512, CH=128, unroll=4, lag=2, skew=0, n_layers=2, flags=None):
    nt = S // TM
    nqb = S // NQ
    nch = S // CH
    nitems = 4 * nqb * 8
    qb_shift = (nqb - 1).bit_length()

    def decode(i):
        h = i & 7
        qb = (i >> 3) & (nqb - 1)
        g = i >> (3 + qb_shift)
        return g, qb, h

    def kernel(x_hbm, wqkv_hbm, wo_hbm, w1_hbm, b1_hbm, w2_hbm, out_hbm,
               xin, xres, wqkv, wqT, wvT, wk, wo, w1, b1, w2,
               k4, qt, vt, ot, s0, s1, qz0, qz1, obuf, sems, osems):
        def x_copy(r):
            return pltpu.make_async_copy(x_hbm.at[pl.ds(r * TM, TM)], xin.at[pl.ds(r * TM, TM)], sems.at[r])

        def o_copy(r):
            rows = pl.ds(pl.multiple_of(r * TM, TM), TM)
            return pltpu.make_async_copy(obuf.at[rows], out_hbm.at[rows], osems.at[r])

        c_wqkv = pltpu.make_async_copy(wqkv_hbm, wqkv, sems.at[nt])
        c_wo = pltpu.make_async_copy(wo_hbm, wo, sems.at[nt + 1])
        c_w1 = pltpu.make_async_copy(w1_hbm, w1, sems.at[nt + 2])
        c_b1 = pltpu.make_async_copy(b1_hbm, b1, sems.at[nt + 3])
        c_w2 = pltpu.make_async_copy(w2_hbm, w2, sems.at[nt + 4])

        c_wqkv.start()
        x_copy(0).start()
        qz0[...] = jnp.zeros(qz0.shape, I32)
        qz1[...] = jnp.zeros(qz1.shape, I32)
        c_wqkv.wait()
        for r in range(1, nt):
            x_copy(r).start()
        c_wo.start()
        c_b1.start()
        c_w1.start()
        c_w2.start()
        wqT[...] = _p32(wqkv[:, 0:D].T)
        wk[...] = _p32(wqkv[:, D:2 * D])
        wvT[...] = _p32(wqkv[:, 2 * D:3 * D].T)

        def qkv_tile(layer, r):
            rows = pl.ds(pl.multiple_of(r * TM, TM), TM)

            @pl.when(layer == 0)
            def _():
                x_copy(r).wait()
                xres[rows, :] = xin[rows, :].astype(F32)

            xn = _layernorm(xres[rows, :]).astype(BF16)
            k = _dot(xn, _u32(wk[...])).astype(BF16)
            half = pl.ds(pl.multiple_of(r * (TM // 2), TM // 2), TM // 2)
            for g in range(4):
                k4[g, half, :] = _p32(k[:, g * 128:(g + 1) * 128])
            cols = pl.ds(pl.multiple_of(r * TM, TM), TM)
            qT = _dot_nt(_u32(wqT[...]), xn) * (LOG2E * DH ** -0.5)
            qt[:, cols] = _p32(qT.astype(BF16))
            vT = _dot_nt(_u32(wvT[...]), xn)
            vt[:, cols] = _p32(vT.astype(BF16))

        def setq(i, qz):
            g, qb, h = decode(i)
            hp = (h + 6) & 7
            qz[pl.ds(pl.multiple_of(hp * 8, 8), 8), :] = jnp.zeros((8, NQ), I32)
            qz[pl.ds(pl.multiple_of(h * 8, 8), 8), :] = qt[
                pl.ds(pl.multiple_of(g * 64 + h * 8, 8), 8), pl.ds(pl.multiple_of(qb * NQ, NQ), NQ)]

        def a_chunk(i, sref, qz, c, m8):
            g, qb, h = decode(i)
            k = _u32(k4[g, pl.ds(c * CH // 2, CH // 2), :])
            s = _dot(k, _u32(qz[...]))
            sref[pl.ds(c * CH, CH), :] = s
            return jnp.maximum(m8, jnp.max(s.reshape(CH // 8, 8, NQ), axis=0))

        def b_chunk(i, sref, m, c, l8, acc, hist):
            g, qb, h = decode(i)
            r0 = c * CH
            s = sref[pl.ds(r0, CH), :]
            mm = m
            if lag > 0 and len(hist) >= lag:
                t = hist[-lag][0:8]
                mm = jnp.minimum(mm, jnp.maximum(mm, t))
            p = jnp.exp2(s.reshape(CH // 8, 8, NQ) - mm[None]).reshape(CH, NQ)
            pb = p.astype(BF16)
            for j in reversed(range(CH // 8)):
                l8 = l8 + p[8 * j:8 * j + 8]
            v = _u32(vt[pl.ds(pl.multiple_of(g * 64 + h * 8, 8), 8), pl.ds(r0, CH)])
            d = _dot(v, pb)
            hist.append(d)
            return l8, acc + d

        def b_fin(i, l8, acc):
            g, qb, h = decode(i)
            l = jnp.sum(l8, axis=0, keepdims=True)
            o = acc / l
            ot[pl.ds(pl.multiple_of(g * 64 + h * 8, 8), 8), pl.ds(pl.multiple_of(qb * NQ, NQ), NQ)] = _p32(o.astype(BF16))

        def m_fin(m8):
            return jnp.broadcast_to(jnp.max(m8, axis=0, keepdims=True), (8, NQ))

        def step(i, m, s_cur, s_nxt, qz, do_a=True, do_b=True):
            hist = []
            m8 = jnp.full((8, NQ), -jnp.inf, F32)
            l8 = jnp.zeros((8, NQ), F32)
            acc = jnp.zeros((16, NQ), F32)
            if do_a:
                setq(i + 1, qz)
            for c in range(nch):
                if do_a:
                    m8 = a_chunk(i + 1, s_nxt, qz, c, m8)
                if do_b:
                    l8, acc = b_chunk(i, s_cur, m, c, l8, acc, hist)
            if do_b:
                b_fin(i, l8, acc)
            return m_fin(m8) if do_a else None

        def attention():
            m = step(-1, None, None, s0, qz0, do_b=False)
            nloop = (nitems - 1) // unroll

            def body(j, m):
                for u in range(unroll):
                    i = unroll * j + u
                    if u % 2 == 0:
                        m = step(i, m, s0, s1, qz1)
                    else:
                        m = step(i, m, s1, s0, qz0)
                return m

            m = lax.fori_loop(0, nloop, body, m)
            for i in range(nloop * unroll, nitems - 1):
                if i % 2 == 0:
                    m = step(i, m, s0, s1, qz1)
                else:
                    m = step(i, m, s1, s0, qz0)
            step(nitems - 1, m, s1 if (nitems - 1) % 2 else s0, None, None, do_a=False)
            qz0[...] = jnp.zeros(qz0.shape, I32)
            qz1[...] = jnp.zeros(qz1.shape, I32)

        def post_tile(layer, r):
            rows = pl.ds(pl.multiple_of(r * TM, TM), TM)
            a = _dot_tn(_u32(ot[:, rows]), wo[...])
            x1 = xres[rows, :] + a
            xn = _layernorm(x1).astype(BF16)
            acc = jnp.zeros((TM, D), F32)
            bias = b1[...].astype(F32).reshape(1, F)
            for j in range(F // FC):
                fc = slice(j * FC, (j + 1) * FC)
                h = _dot(xn, w1[:, fc]) + bias[:, fc]
                acc = acc + _dot(_mish(h).astype(BF16), w2[fc, :])
            x2 = x1 + acc
            xres[rows, :] = x2

            @pl.when(layer == n_layers - 1)
            def _():
                obuf[rows, :] = x2.astype(BF16)
                o_copy(r).start()

        def layer_body(layer, carry):
            lax.fori_loop(0, nt, lambda r, c: (qkv_tile(layer, r), c)[1], 0)
            attention()

            @pl.when(layer == 0)
            def _():
                c_wo.wait()
                c_b1.wait()
                c_w1.wait()
                c_w2.wait()

            lax.fori_loop(0, nt, lambda r, c: (post_tile(layer, r), c)[1], 0)
            return carry

        lax.fori_loop(0, n_layers, layer_body, 0)
        for r in range(nt):
            o_copy(r).wait()

    any_spec = pl.BlockSpec(memory_space=pl.ANY)

    def f(x, wqkv, wo, w1, b1, w2):
        VM = pltpu.VMEM
        return pl.pallas_call(
            kernel,
            out_shape=jax.ShapeDtypeStruct((S, D), BF16),
            in_specs=[any_spec] * 6,
            out_specs=any_spec,
            scratch_shapes=[
                VM((S, D), BF16),
                VM((S, D), F32),
                VM((D, 3 * D), BF16),
                VM((D // 2, D), I32),
                VM((D // 2, D), I32),
                VM((D // 2, D), I32),
                VM((D, D), BF16),
                VM((D, F), BF16),
                VM((F,), BF16),
                VM((F, D), BF16),
                VM((4, S // 2, 128), I32),
                VM((D // 2, S), I32),
                VM((D // 2, S), I32),
                VM((D // 2, S), I32),
                VM((S, NQ), F32),
                VM((S, NQ), F32),
                VM((64, NQ), I32),
                VM((64, NQ), I32),
                VM((S, D), BF16),
                pltpu.SemaphoreType.DMA((nt + 5,)),
                pltpu.SemaphoreType.DMA((nt,)),
            ],
            compiler_params=pltpu.CompilerParams(vmem_limit_bytes=100 * 1024 * 1024, flags=flags),
        )(x, wqkv, wo, w1, b1, w2)

    return f


@jax.jit
def pallas_interleave_layers__mha_block__dense_activation_mish__prompt_kernel(
    A_x, A_wqkv, A_wo, B_x, B_w1, B_b1, B_w2,
):
    del B_x
    out = make()(A_x.reshape(S, D), A_wqkv, A_wo, B_w1, B_b1, B_w2)
    return out.reshape(1, S, D)
```

```python
import functools
import math

import jax
import jax.numpy as jnp
import numpy as np
from jax import lax
import jax.experimental.pallas as pl
import jax.experimental.pallas.tpu as pltpu

S, D, H, DH, F = 2048, 512, 32, 16, 1792
LOG2E = 1.4426950408889634
EPS = 1e-5
BF16, F32, I32 = jnp.bfloat16, jnp.float32, jnp.int32


def _dot(a, b):
    return jnp.dot(a, b, preferred_element_type=F32)


def _dot_nt(a, b):
    return lax.dot_general(a, b, (((1,), (1,)), ((), ())), preferred_element_type=F32)


def _dot_tn(a, b):
    return lax.dot_general(a, b, (((0,), (0,)), ((), ())), preferred_element_type=F32)


def _p32(x):
    return pltpu.bitcast(x, I32)


def _u32(x):
    return pltpu.bitcast(x, BF16)


def _layernorm(x):
    m = jnp.mean(x, axis=-1, keepdims=True)
    xc = x - m
    v = jnp.mean(xc * xc, axis=-1, keepdims=True)
    return xc * lax.rsqrt(v + EPS)


def _mish_ref(h):
    sp = jnp.log1p(jnp.exp(-jnp.abs(h))) + jnp.maximum(h, 0.0)
    return h * jnp.tanh(sp)


def _mish(h):
    e = jnp.exp2(jnp.minimum(h, 20.0) * LOG2E)
    n = e * (e + 2.0)
    return (h * n) * pltpu.reciprocal(n + 2.0, approx=True)


def make(TM=512, NS=4, NK1=2, FC=256, NQ=512, CH=128, unroll=12, lag=3, skew=1, boff=8, n_layers=2, flags=None, only_attn=False):
    nt = S // TM
    TS = TM // NS
    nqb = S // NQ
    nch = S // CH
    nitems = 4 * nqb * 8
    qb_shift = (nqb - 1).bit_length()

    def decode(i):
        h = i & 7
        qb = (i >> 3) & (nqb - 1)
        g = i >> (3 + qb_shift)
        return g, qb, h

    def kernel(x_hbm, wqkv_hbm, wo_hbm, w1_hbm, b1_hbm, w2_hbm, out_hbm,
               xin, xres, wq_raw, wv_raw, wqT, wvT, wk, wo, w1, b1, w2,
               k4, qt, vt, ot, s0, s1, qz0, qz1, obuf, sems, osems):
        def x_copy(r):
            return pltpu.make_async_copy(x_hbm.at[pl.ds(r * TM, TM)], xin.at[pl.ds(r * TM, TM)], sems.at[r])

        def o_copy(r, u):
            rows = pl.ds(pl.multiple_of(r * TM + u * TS, TS), TS)
            return pltpu.make_async_copy(obuf.at[rows], out_hbm.at[rows], osems.at[r * NS + u])

        c_wq = pltpu.make_async_copy(wqkv_hbm.at[:, pl.ds(0, D)], wq_raw, sems.at[nt])
        c_wk = pltpu.make_async_copy(wqkv_hbm.at[:, pl.ds(D, D)], wk, sems.at[nt + 1])
        c_wv = pltpu.make_async_copy(wqkv_hbm.at[:, pl.ds(2 * D, D)], wv_raw, sems.at[nt + 2])
        c_wo = pltpu.make_async_copy(wo_hbm, wo, sems.at[nt + 3])
        c_w1 = pltpu.make_async_copy(w1_hbm, w1, sems.at[nt + 4])
        c_b1 = pltpu.make_async_copy(b1_hbm, b1, sems.at[nt + 5])
        c_w2 = pltpu.make_async_copy(w2_hbm, w2, sems.at[nt + 6])

        x_copy(0).start()
        c_wk.start()
        x_copy(1).start()
        c_wq.start()
        c_wv.start()
        for r in range(2, nt):
            x_copy(r).start()
        c_wo.start()
        c_b1.start()
        c_w1.start()
        c_w2.start()
        qz0[...] = jnp.zeros(qz0.shape, I32)
        qz1[...] = jnp.zeros(qz1.shape, I32)

        def sub_rows(r0, u, n=TS):
            return pl.ds(pl.multiple_of(r0 + u * TS, TS), n)

        def qkv_dots(xn, r0, u):
            def k_part():
                k = _dot(xn, wk[...]).astype(BF16)
                half = pl.ds(pl.multiple_of((r0 + u * TS) // 2, TS // 2), TS // 2)
                for g in range(4):
                    k4[g, half, :] = _p32(k[:, g * 128:(g + 1) * 128])

            def q_part():
                qT = _dot_nt(_u32(wqT[...]), xn) * (LOG2E * DH ** -0.5)
                qt[:, sub_rows(r0, u)] = _p32(qT.astype(BF16))

            def v_part():
                vT = _dot_nt(_u32(wvT[...]), xn)
                vt[:, sub_rows(r0, u)] = _p32(vT.astype(BF16))

            return [k_part, q_part, v_part]

        def qkv_first():
            parts = {}

            def ln(r, us=None):
                for u in (range(NS) if us is None else us):
                    x = xin[sub_rows(r * TM, u), :].astype(F32)
                    xres[sub_rows(r * TM, u), :] = x
                    parts[r, u] = qkv_dots(_layernorm(x).astype(BF16), r * TM, u)

            hs = NS // 2
            x_copy(0).wait()
            ln(0, [0])
            c_wk.wait()
            ln(0, range(1, NS))
            for u in range(hs):
                parts[0, u][0]()
            x_copy(1).wait()
            ln(1)
            for u in range(hs, NS):
                parts[0, u][0]()
            for u in range(hs):
                parts[1, u][0]()
            c_wq.wait()
            c_wv.wait()
            wqT[...] = _p32(wq_raw[...].T)
            wvT[...] = _p32(wv_raw[...].T)
            for u in range(hs, NS):
                parts[1, u][0]()
            for u in range(NS):
                parts[0, u][1]()
                parts[0, u][2]()
            for r in range(2, nt):
                x_copy(r).wait()
            for r in range(2, nt):
                ln(r)
            for u in range(NS):
                parts[1, u][1]()
                parts[1, u][2]()
            for r in range(2, nt):
                for u in range(NS):
                    for t in parts[r, u]:
                        t()

        def setq(i, qz):
            g, qb, h = decode(i)
            hp = (h + 6) & 7
            qz[pl.ds(pl.multiple_of(hp * 8, 8), 8), :] = jnp.zeros((8, NQ), I32)
            qz[pl.ds(pl.multiple_of(h * 8, 8), 8), :] = qt[
                pl.ds(pl.multiple_of(g * 64 + h * 8, 8), 8), pl.ds(pl.multiple_of(qb * NQ, NQ), NQ)]

        def a_chunk(i, sref, qz, c, m8):
            g, qb, h = decode(i)
            k = _u32(k4[g, pl.ds(c * CH // 2, CH // 2), :])
            s = _dot(k, _u32(qz[...]))
            sref[pl.ds(c * CH, CH), :] = s
            return jnp.maximum(m8, jnp.max(s.reshape(CH // 8, 8, NQ), axis=0))

        def b_chunk(i, sref, m, c, l8, acc, hist):
            g, qb, h = decode(i)
            r0 = c * CH
            s = sref[pl.ds(r0, CH), :]
            mm = m
            if lag > 0 and len(hist) >= lag:
                t = hist[-lag][0:8]
                mm = jnp.minimum(mm, jnp.maximum(mm, t))
            p = jnp.exp2(s.reshape(CH // 8, 8, NQ) - mm[None]).reshape(CH, NQ)
            pb = p.astype(BF16)
            for j in reversed(range(CH // 8)):
                l8 = l8 + p[8 * j:8 * j + 8]
            v = _u32(vt[pl.ds(pl.multiple_of(g * 64 + h * 8, 8), 8), pl.ds(r0, CH)])
            d = _dot(v, pb)
            hist.append(d)
            return l8, acc + d

        def b_fin(i, l8, acc):
            g, qb, h = decode(i)
            l = jnp.sum(l8, axis=0, keepdims=True)
            o = acc / l
            ot[pl.ds(pl.multiple_of(g * 64 + h * 8, 8), 8), pl.ds(pl.multiple_of(qb * NQ, NQ), NQ)] = _p32(o.astype(BF16))

        def m_fin(m8):
            return jnp.broadcast_to(jnp.max(m8, axis=0, keepdims=True), (8, NQ))

        class St:
            pass

        def run_stream(ib, a_lo, a_hi, st, nA, lagc):
            hist = []
            for a in range(a_lo, a_hi):
                if nA is None or a < nA:
                    di, c = divmod(a, nch)
                    sref, qz = (s0, qz0) if di % 2 == 0 else (s1, qz1)
                    if c == 0:
                        setq(ib + di, qz)
                        st.m8 = jnp.full((8, NQ), -jnp.inf, F32)
                    st.m8 = a_chunk(ib + di, sref, qz, c, st.m8)
                    if c == nch - 1:
                        st.m_next = m_fin(st.m8)
                        st.m8 = None
                b = a - lagc
                if b >= st.b_lo:
                    di, c = divmod(b, nch)
                    sref = s0 if di % 2 == 0 else s1
                    if c == 0:
                        st.m = st.mq.pop(0) if st.mq else None
                        st.l8 = jnp.zeros((8, NQ), F32)
                        st.acc = jnp.zeros((16, NQ), F32)
                    st.l8, st.acc = b_chunk(ib + di, sref, st.m, c, st.l8, st.acc, hist)
                    if c == nch - 1:
                        b_fin(ib + di, st.l8, st.acc)
                if st.m8 is None and st.m_next is not None:
                    st.mq.append(st.m_next)
                    st.m_next = None

        def attention(first):
            lagc = nch + skew
            per = unroll * nch
            ntot = nitems * nch
            a0 = lagc + boff
            nloop = (ntot - a0) // per
            st = St()
            st.mq, st.m8, st.m_next, st.b_lo = [], None, None, 0
            st.m = st.l8 = st.acc = None
            run_stream(0, 0, a0, st, None, lagc)
            in_a = a0 % nch != 0
            in_b = (a0 - lagc) % nch != 0
            nq = len(st.mq)

            def pack(s):
                return (tuple(s.mq), s.m8 if in_a else None, (s.m, s.l8, s.acc) if in_b else None)

            def unpack(carry):
                s = St()
                s.mq, s.m8, s.m_next, s.b_lo = list(carry[0]), carry[1], None, 0
                s.m, s.l8, s.acc = carry[2] if in_b else (None, None, None)
                return s

            def body(j, carry):
                s = unpack(carry)
                run_stream(j * unroll, a0, a0 + per, s, None, lagc)
                return pack(s)

            carry = lax.fori_loop(0, nloop, body, pack(st))
            if first:
                c_wo.wait()
                c_b1.wait()
                c_w1.wait()
                c_w2.wait()
            a_end = ntot - nloop * per
            run_stream(nloop * unroll, a0, a_end + lagc, unpack(carry), a_end, lagc)
            qz0[...] = jnp.zeros(qz0.shape, I32)
            qz1[...] = jnp.zeros(qz1.shape, I32)

        def post_tile(r, last):
            r0 = r * TM
            nj = F // FC
            bias = b1[...].astype(F32).reshape(1, F)
            a = [_dot_tn(_u32(ot[:, sub_rows(r0, u)]), wo[...]) for u in range(NS)]
            x1 = [xres[sub_rows(r0, u), :] + a[u] for u in range(NS)]
            xn = [_layernorm(x1[u]).astype(BF16) for u in range(NS)]
            acc = [None] * NS
            hs = {}
            pending = []

            def f1(u, j):
                fc = slice(j * FC, (j + 1) * FC)
                hs[u, j] = _dot(xn[u], w1[:, fc]) + bias[:, fc]

            def f2(u, j):
                fc = slice(j * FC, (j + 1) * FC)
                d = _dot(_mish(hs.pop((u, j))).astype(BF16), w2[fc, :])
                acc[u] = d if acc[u] is None else acc[u] + d
                if j == nj - 1:
                    x2 = x1[u] + acc[u]
                    if last:
                        obuf[sub_rows(r0, u), :] = x2.astype(BF16)
                        o_copy(r, u).start()
                    else:
                        xres[sub_rows(r0, u), :] = x2
                        pending.extend(qkv_dots(_layernorm(x2).astype(BF16), r0, u))

            tasks = [(u, j) for u in range(NS) for j in range(nj)]
            f1(*tasks[0])
            for n, t in enumerate(tasks):
                if n + 1 < len(tasks):
                    f1(*tasks[n + 1])
                elif pending:
                    pending.pop(0)()
                f2(*t)
            while pending:
                pending.pop(0)()

        qkv_first()
        for layer in range(n_layers):
            attention(layer == 0)
            last = layer == n_layers - 1
            lax.fori_loop(0, nt, lambda r, c, last=last: (post_tile(r, last), c)[1], 0)
        for r in range(nt):
            for u in range(NS):
                o_copy(r, u).wait()

    any_spec = pl.BlockSpec(memory_space=pl.ANY)

    def f(x, wqkv, wo, w1, b1, w2):
        VM = pltpu.VMEM
        return pl.pallas_call(
            kernel,
            out_shape=jax.ShapeDtypeStruct((S, D), BF16),
            in_specs=[any_spec] * 6,
            out_specs=any_spec,
            scratch_shapes=[
                VM((S, D), BF16),
                VM((S, D), F32),
                VM((D, D), BF16),
                VM((D, D), BF16),
                VM((D // 2, D), I32),
                VM((D // 2, D), I32),
                VM((D, D), BF16),
                VM((D, D), BF16),
                VM((D, F), BF16),
                VM((F,), BF16),
                VM((F, D), BF16),
                VM((4, S // 2, 128), I32),
                VM((D // 2, S), I32),
                VM((D // 2, S), I32),
                VM((D // 2, S), I32),
                VM((S, NQ), F32),
                VM((S, NQ), F32),
                VM((64, NQ), I32),
                VM((64, NQ), I32),
                VM((S, D), BF16),
                pltpu.SemaphoreType.DMA((nt + 7,)),
                pltpu.SemaphoreType.DMA((nt * NS,)),
            ],
            compiler_params=pltpu.CompilerParams(vmem_limit_bytes=100 * 1024 * 1024, flags=flags),
        )(x, wqkv, wo, w1, b1, w2)

    return f


@jax.jit
def pallas_interleave_layers__mha_block__dense_activation_mish__prompt_kernel(
    A_x, A_wqkv, A_wo, B_x, B_w1, B_b1, B_w2,
):
    del B_x
    out = make()(A_x.reshape(S, D), A_wqkv, A_wo, B_w1, B_b1, B_w2)
    return out.reshape(1, S, D)
```

```python
import jax
import jax.numpy as jnp
from jax import lax
import jax.experimental.pallas as pl
import jax.experimental.pallas.tpu as pltpu

S, D, H, DH, F = 2048, 512, 32, 16, 1792
LOG2E = 1.4426950408889634
EPS = 1e-5
BF16, F32, I32 = jnp.bfloat16, jnp.float32, jnp.int32
HD, HF = D // 2, F // 2


def _dot(a, b):
    return jnp.dot(a, b, preferred_element_type=F32)


def _dot_nt(a, b):
    return lax.dot_general(a, b, (((1,), (1,)), ((), ())), preferred_element_type=F32)


def _dot_tn(a, b):
    return lax.dot_general(a, b, (((0,), (0,)), ((), ())), preferred_element_type=F32)


def _p32(x):
    return pltpu.bitcast(x, I32)


def _u32(x):
    return pltpu.bitcast(x, BF16)


def _layernorm(x):
    m = jnp.mean(x, axis=-1, keepdims=True)
    xc = x - m
    v = jnp.mean(xc * xc, axis=-1, keepdims=True)
    return xc * lax.rsqrt(v + EPS)


def _mish(h):
    e = jnp.exp2(jnp.minimum(h, 20.0) * LOG2E)
    n = e * (e + 2.0)
    return (h * n) * pltpu.reciprocal(n + 2.0, approx=True)


def _st_a(a11, a12, a21, a22):
    return [a11 + a22, a21 + a22, a11, a22, a11 + a12, a21 - a11, a12 - a22]


def _st_b(b11, b12, b21, b22):
    return [b11 + b22, b11, b12 - b22, b21 - b11, b22, b11 + b12, b21 + b22]


def _st_c(m):
    return (m[0] + m[3] - m[4] + m[6], m[2] + m[4], m[1] + m[3], m[0] - m[1] + m[2] + m[5])


def make(TM=512, NQ=512, CH=128, unroll=12, lag=3, skew=1, boff=8, PR=32, n_layers=2, flags=None, st_wo=False):
    nt = S // TM
    NP = TM // 256
    npair = S // 256
    nqb = S // NQ
    nch = S // CH
    nitems = 4 * nqb * 8
    qb_shift = (nqb - 1).bit_length()

    def decode(i):
        h = i & 7
        qb = (i >> 3) & (nqb - 1)
        g = i >> (3 + qb_shift)
        return g, qb, h

    def kernel(x_hbm, wqkv_hbm, wo_hbm, w1_hbm, b1_hbm, w2_hbm, out_hbm,
               xin, xres, wq, wk, wv, wo, w1, b1, w2, wqc, wkc, wvc, w1c, w2c,
               k4, qt, vt, ot, s0, s1, qz0, qz1, obuf, xsems, wsems, osems):
        def half_rows(row0, t):
            return pl.ds(pl.multiple_of(row0 + t * 128, 128), 128)

        def x_copy(p):
            rows = pl.ds(p * 256, 256)
            return pltpu.make_async_copy(x_hbm.at[rows], xin.at[rows], xsems.at[p])

        def o_copy(p, t):
            rows = half_rows(p * 256, t)
            return pltpu.make_async_copy(obuf.at[rows], out_hbm.at[rows], osems.at[2 * p + t])

        c_wq = pltpu.make_async_copy(wqkv_hbm.at[:, pl.ds(0, D)], wq, wsems.at[0])
        c_wk = pltpu.make_async_copy(wqkv_hbm.at[:, pl.ds(D, D)], wk, wsems.at[1])
        c_wv = pltpu.make_async_copy(wqkv_hbm.at[:, pl.ds(2 * D, D)], wv, wsems.at[2])
        c_wo = pltpu.make_async_copy(wo_hbm, wo, wsems.at[3])
        c_w1 = pltpu.make_async_copy(w1_hbm, w1, wsems.at[4])
        c_b1 = pltpu.make_async_copy(b1_hbm, b1, wsems.at[5])
        c_w2 = pltpu.make_async_copy(w2_hbm, w2, wsems.at[6])

        x_copy(0).start()
        c_wk.start()
        for p in (1, 2, 3):
            x_copy(p).start()
        c_wq.start()
        c_wv.start()
        for p in range(4, npair):
            x_copy(p).start()
        c_wo.start()
        c_b1.start()
        c_w1.start()
        c_w2.start()
        qz0[...] = jnp.zeros(qz0.shape, I32)
        qz1[...] = jnp.zeros(qz1.shape, I32)

        def prep_pieces(dst, load, hr, hc, transposed=False):
            def piece(r, c):
                def run():
                    raw = [load(r, PR, c), load(r, PR, hc + c), load(hr + r, PR, c), load(hr + r, PR, hc + c)]
                    if transposed:
                        raw[1], raw[2] = raw[2], raw[1]
                    for i, t in enumerate(_st_b(*[t.astype(F32) for t in raw])):
                        t = raw[0] if i == 1 else raw[3] if i == 4 else t.astype(BF16)
                        dst[i, r // 2:(r + PR) // 2, c:c + 128] = _p32(t)
                return run
            return [piece(r, c) for r in range(0, hr, PR) for c in range(0, hc, 128)]

        def ref_loader(w):
            return lambda r, n, c: w[r:r + n, c:c + 128]

        def prep_transposed(dst, w):
            wt = w[...].T
            for t in prep_pieces(dst, lambda r, n, c: wt[r:r + n, c:c + 128], HD, HD, True):
                t()

        def qkv_dots(xn_top, xn_bot, row0):
            xc = [c.astype(BF16) for c in _st_a(xn_top[:, :HD], xn_top[:, HD:], xn_bot[:, :HD], xn_bot[:, HD:])]

            def k_part():
                c11, c12, c21, c22 = _st_c([_dot(xc[i], _u32(wkc[i])) for i in range(7)])
                for t, (cl, cr) in enumerate(((c11, c12), (c21, c22))):
                    rows = pl.ds(pl.multiple_of((row0 + t * 128) // 2, 64), 64)
                    for g, blk in enumerate((cl[:, :128], cl[:, 128:], cr[:, :128], cr[:, 128:])):
                        k4[g, rows, :] = _p32(blk.astype(BF16))

            def t_part(wc, dst, scale):
                def run():
                    c11, c12, c21, c22 = _st_c([_dot_nt(_u32(wc[i]), xc[i]) for i in range(7)])
                    for t, (cl, cr) in enumerate(((c11, c12), (c21, c22))):
                        for o, blk in enumerate((cl, cr)):
                            blk = blk if scale is None else blk * scale
                            dst[o * 128:(o + 1) * 128, half_rows(row0, t)] = _p32(blk.astype(BF16))
                return run

            return [k_part, t_part(wqc, qt, LOG2E * DH ** -0.5), t_part(wvc, vt, None)]

        def qkv_first():
            parts = {}

            def ln(p):
                xn = []
                for t in range(2):
                    x = xin[half_rows(p * 256, t), :].astype(F32)
                    xres[half_rows(p * 256, t), :] = x
                    xn.append(_layernorm(x))
                parts[p] = qkv_dots(xn[0], xn[1], p * 256)

            x_copy(0).wait()
            ln(0)
            c_wk.wait()
            for t in prep_pieces(wkc, ref_loader(wk), HD, HD):
                t()
            x_copy(1).wait()
            parts[0][0]()
            ln(1)
            x_copy(2).wait()
            x_copy(3).wait()
            parts[1][0]()
            ln(2)
            ln(3)
            parts[2][0]()
            c_wq.wait()
            c_wv.wait()
            prep_transposed(wqc, wq)
            parts[3][0]()
            prep_transposed(wvc, wv)
            for p in (0, 1, 2):
                parts[p][1]()
            for p in (0, 1, 2):
                parts[p][2]()
            for p in range(4, npair):
                x_copy(p).wait()
            for p in range(4, npair):
                ln(p)
            parts[3][1]()
            parts[3][2]()
            for p in range(4, npair):
                for t in parts[p]:
                    t()

        def setq(i, qz):
            g, qb, h = decode(i)
            hp = (h + 6) & 7
            qz[pl.ds(pl.multiple_of(hp * 8, 8), 8), :] = jnp.zeros((8, NQ), I32)
            qz[pl.ds(pl.multiple_of(h * 8, 8), 8), :] = qt[
                pl.ds(pl.multiple_of(g * 64 + h * 8, 8), 8), pl.ds(pl.multiple_of(qb * NQ, NQ), NQ)]

        def a_chunk(i, sref, qz, c, m8):
            g, qb, h = decode(i)
            k = _u32(k4[g, pl.ds(c * CH // 2, CH // 2), :])
            s = _dot(k, _u32(qz[...]))
            sref[pl.ds(c * CH, CH), :] = s
            return jnp.maximum(m8, jnp.max(s.reshape(CH // 8, 8, NQ), axis=0))

        def b_chunk(i, sref, m, c, l8, acc, hist):
            g, qb, h = decode(i)
            r0 = c * CH
            s = sref[pl.ds(r0, CH), :]
            mm = m
            if len(hist) >= lag:
                t = hist[-lag][0:8]
                mm = jnp.minimum(mm, jnp.maximum(mm, t))
            p = jnp.exp2(s.reshape(CH // 8, 8, NQ) - mm[None]).reshape(CH, NQ)
            pb = p.astype(BF16)
            for j in reversed(range(CH // 8)):
                l8 = l8 + p[8 * j:8 * j + 8]
            v = _u32(vt[pl.ds(pl.multiple_of(g * 64 + h * 8, 8), 8), pl.ds(r0, CH)])
            d = _dot(v, pb)
            hist.append(d)
            return l8, acc + d

        def b_fin(i, l8, acc):
            g, qb, h = decode(i)
            l = jnp.sum(l8, axis=0, keepdims=True)
            o = acc / l
            ot[pl.ds(pl.multiple_of(g * 64 + h * 8, 8), 8), pl.ds(pl.multiple_of(qb * NQ, NQ), NQ)] = _p32(o.astype(BF16))

        def m_fin(m8):
            return jnp.broadcast_to(jnp.max(m8, axis=0, keepdims=True), (8, NQ))

        class St:
            pass

        def run_stream(ib, a_lo, a_hi, st, nA, lagc, filler=None):
            hist = []
            nfill = -(-len(filler) // (a_hi - a_lo)) if filler else 0
            for a in range(a_lo, a_hi):
                if nA is None or a < nA:
                    di, c = divmod(a, nch)
                    sref, qz = (s0, qz0) if di % 2 == 0 else (s1, qz1)
                    if c == 0:
                        setq(ib + di, qz)
                        st.m8 = jnp.full((8, NQ), -jnp.inf, F32)
                    st.m8 = a_chunk(ib + di, sref, qz, c, st.m8)
                    if c == nch - 1:
                        st.m_next = m_fin(st.m8)
                        st.m8 = None
                    for _ in range(nfill):
                        if filler:
                            filler.pop(0)()
                b = a - lagc
                if b >= 0:
                    di, c = divmod(b, nch)
                    sref = s0 if di % 2 == 0 else s1
                    if c == 0:
                        st.m = st.mq.pop(0)
                        st.l8 = jnp.zeros((8, NQ), F32)
                        st.acc = jnp.zeros((16, NQ), F32)
                    st.l8, st.acc = b_chunk(ib + di, sref, st.m, c, st.l8, st.acc, hist)
                    if c == nch - 1:
                        b_fin(ib + di, st.l8, st.acc)
                if st.m8 is None and st.m_next is not None:
                    st.mq.append(st.m_next)
                    st.m_next = None

        def attention(first):
            lagc = nch + skew
            per = unroll * nch
            ntot = nitems * nch
            a0 = lagc + boff
            nloop = (ntot - a0) // per
            st = St()
            st.mq, st.m8, st.m_next = [], None, None
            st.m = st.l8 = st.acc = None
            filler = None
            if first:
                c_wo.wait()
                c_b1.wait()
                c_w1.wait()
                c_w2.wait()
                filler = prep_pieces(w1c, ref_loader(w1), HD, HF) + prep_pieces(w2c, ref_loader(w2), HF, HD)
            run_stream(0, 0, a0, st, None, lagc, filler)
            assert not filler
            in_a = a0 % nch != 0
            in_b = (a0 - lagc) % nch != 0

            def pack(s):
                return (tuple(s.mq), s.m8 if in_a else None, (s.m, s.l8, s.acc) if in_b else None)

            def unpack(carry):
                s = St()
                s.mq, s.m8, s.m_next = list(carry[0]), carry[1], None
                s.m, s.l8, s.acc = carry[2] if in_b else (None, None, None)
                return s

            def body(j, carry):
                s = unpack(carry)
                run_stream(j * unroll, a0, a0 + per, s, None, lagc)
                return pack(s)

            carry = lax.fori_loop(0, nloop, body, pack(st))
            a_end = ntot - nloop * per
            run_stream(nloop * unroll, a0, a_end + lagc, unpack(carry), a_end, lagc)
            qz0[...] = jnp.zeros(qz0.shape, I32)
            qz1[...] = jnp.zeros(qz1.shape, I32)

        NJ = HF // 128

        def post_tile(r, last):
            r0 = r * TM
            bias = b1[...].astype(F32).reshape(1, F)
            hv = [(p, t) for p in range(NP) for t in range(2)]
            a = {k: _dot_tn(_u32(ot[:, half_rows(r0 + k[0] * 256, k[1])]), wo[...]) for k in hv}
            x1 = {k: xres[half_rows(r0 + k[0] * 256, k[1]), :] + a[k] for k in hv}
            xn = {k: _layernorm(x1[k]) for k in hv}
            xc = [[c.astype(BF16) for c in _st_a(xn[p, 0][:, :HD], xn[p, 0][:, HD:], xn[p, 1][:, :HD], xn[p, 1][:, HD:])]
                  for p in range(NP)]
            acc = [None] * NP
            hs = {}
            pending = []

            def f1(p, j):
                c0 = slice(j * 128, (j + 1) * 128)
                c1 = slice(HF + j * 128, HF + (j + 1) * 128)
                c11, c12, c21, c22 = _st_c([_dot(xc[p][i], _u32(w1c[i, :, c0])) for i in range(7)])
                hs[p, j] = (c11 + bias[:, c0], c12 + bias[:, c1], c21 + bias[:, c0], c22 + bias[:, c1])

            def f2(p, j):
                acts = [_mish(t) for t in hs.pop((p, j))]
                m = [_dot(t.astype(BF16), _u32(w2c[i, j * 64:(j + 1) * 64, :])) for i, t in enumerate(_st_a(*acts))]
                acc[p] = m if acc[p] is None else [x + y for x, y in zip(acc[p], m)]
                if j == NJ - 1:
                    c11, c12, c21, c22 = _st_c(acc[p])
                    x2 = [x1[p, t] + jnp.concatenate(cc, axis=1) for t, cc in enumerate(((c11, c12), (c21, c22)))]
                    for t in range(2):
                        rows = half_rows(r0 + p * 256, t)
                        if last:
                            obuf[rows, :] = x2[t].astype(BF16)
                            o_copy(r * NP + p, t).start()
                        else:
                            xres[rows, :] = x2[t]
                    if not last:
                        pending.extend(qkv_dots(_layernorm(x2[0]), _layernorm(x2[1]), r0 + p * 256))

            tasks = [(p, j) for p in range(NP) for j in range(NJ)]
            f1(*tasks[0])
            for n, t in enumerate(tasks):
                if n + 1 < len(tasks):
                    f1(*tasks[n + 1])
                elif pending:
                    pending.pop(0)()
                f2(*t)
            while pending:
                pending.pop(0)()

        qkv_first()
        for layer in range(n_layers):
            attention(layer == 0)
            last = layer == n_layers - 1
            lax.fori_loop(0, nt, lambda r, c, last=last: (post_tile(r, last), c)[1], 0)
        for p in range(npair):
            for t in range(2):
                o_copy(p, t).wait()

    any_spec = pl.BlockSpec(memory_space=pl.ANY)

    def f(x, wqkv, wo, w1, b1, w2):
        VM = pltpu.VMEM
        return pl.pallas_call(
            kernel,
            out_shape=jax.ShapeDtypeStruct((S, D), BF16),
            in_specs=[any_spec] * 6,
            out_specs=any_spec,
            scratch_shapes=[
                VM((S, D), BF16),
                VM((S, D), F32),
                VM((D, D), BF16),
                VM((D, D), BF16),
                VM((D, D), BF16),
                VM((D, D), BF16),
                VM((D, F), BF16),
                VM((F,), BF16),
                VM((F, D), BF16),
                VM((7, HD // 2, HD), I32),
                VM((7, HD // 2, HD), I32),
                VM((7, HD // 2, HD), I32),
                VM((7, HD // 2, HF), I32),
                VM((7, HF // 2, HD), I32),
                VM((4, S // 2, 128), I32),
                VM((D // 2, S), I32),
                VM((D // 2, S), I32),
                VM((D // 2, S), I32),
                VM((S, NQ), F32),
                VM((S, NQ), F32),
                VM((64, NQ), I32),
                VM((64, NQ), I32),
                VM((S, D), BF16),
                pltpu.SemaphoreType.DMA((npair,)),
                pltpu.SemaphoreType.DMA((7,)),
                pltpu.SemaphoreType.DMA((2 * npair,)),
            ],
            compiler_params=pltpu.CompilerParams(vmem_limit_bytes=100 * 1024 * 1024, flags=flags),
        )(x, wqkv, wo, w1, b1, w2)

    return f


@jax.jit
def pallas_interleave_layers__mha_block__dense_activation_mish__prompt_kernel(
    A_x, A_wqkv, A_wo, B_x, B_w1, B_b1, B_w2,
):
    del B_x
    out = make()(A_x.reshape(S, D), A_wqkv, A_wo, B_w1, B_b1, B_w2)
    return out.reshape(1, S, D)
```

```python
import jax
import jax.numpy as jnp
from jax import lax
import jax.experimental.pallas as pl
import jax.experimental.pallas.tpu as pltpu

S, D, H, DH, F = 2048, 512, 32, 16, 1792
HD, HF = D // 2, F // 2
LOG2E = 1.4426950408889634
EPS = 1e-5
BF16, F32, I32 = jnp.bfloat16, jnp.float32, jnp.int32

N_LAYERS = 2
TM = 512
NT = S // TM
NP = TM // 256
NPAIR = S // 256
NQ = 512
NQB = S // NQ
CH = 128
NCH = S // CH
NITEMS = 4 * NQB * 8
UNROLL = 12
LAG = 3
LAGC = NCH + 1
A0 = LAGC + 8
PR = 32


def _dot(a, b):
    return jnp.dot(a, b, preferred_element_type=F32)


def _dot_nt(a, b):
    return lax.dot_general(a, b, (((1,), (1,)), ((), ())), preferred_element_type=F32)


def _dot_tn(a, b):
    return lax.dot_general(a, b, (((0,), (0,)), ((), ())), preferred_element_type=F32)


def _p32(x):
    return pltpu.bitcast(x, I32)


def _u32(x):
    return pltpu.bitcast(x, BF16)


def _layernorm(x):
    m = jnp.mean(x, axis=-1, keepdims=True)
    xc = x - m
    v = jnp.mean(xc * xc, axis=-1, keepdims=True)
    return xc * lax.rsqrt(v + EPS)


def _mish(h):
    e = jnp.exp2(jnp.minimum(h, 20.0) * LOG2E)
    n = e * (e + 2.0)
    return (h * n) * pltpu.reciprocal(n + 2.0, approx=True)


def _st_a(a11, a12, a21, a22):
    return [a11 + a22, a21 + a22, a11, a22, a11 + a12, a21 - a11, a12 - a22]


def _st_b(b11, b12, b21, b22):
    return [b11 + b22, b11, b12 - b22, b21 - b11, b22, b11 + b12, b21 + b22]


def _st_c(m):
    return (m[0] + m[3] - m[4] + m[6], m[2] + m[4], m[1] + m[3], m[0] - m[1] + m[2] + m[5])


def _decode(i):
    return i >> (3 + (NQB - 1).bit_length()), (i >> 3) & (NQB - 1), i & 7


class _Stream:
    pass


def _kernel(x_hbm, wqkv_hbm, wo_hbm, w1_hbm, b1_hbm, w2_hbm, out_hbm,
            xin, xres, wq, wk, wv, wo, w1, b1, w2, wqc, wkc, wvc, w1c, w2c,
            k4, qt, vt, ot, s0, s1, qz0, qz1, obuf, xsems, wsems, osems):
    def half_rows(row0, t):
        return pl.ds(pl.multiple_of(row0 + t * 128, 128), 128)

    def x_copy(p):
        rows = pl.ds(p * 256, 256)
        return pltpu.make_async_copy(x_hbm.at[rows], xin.at[rows], xsems.at[p])

    def o_copy(p, t):
        rows = half_rows(p * 256, t)
        return pltpu.make_async_copy(obuf.at[rows], out_hbm.at[rows], osems.at[2 * p + t])

    c_wq = pltpu.make_async_copy(wqkv_hbm.at[:, pl.ds(0, D)], wq, wsems.at[0])
    c_wk = pltpu.make_async_copy(wqkv_hbm.at[:, pl.ds(D, D)], wk, wsems.at[1])
    c_wv = pltpu.make_async_copy(wqkv_hbm.at[:, pl.ds(2 * D, D)], wv, wsems.at[2])
    c_wo = pltpu.make_async_copy(wo_hbm, wo, wsems.at[3])
    c_w1 = pltpu.make_async_copy(w1_hbm, w1, wsems.at[4])
    c_b1 = pltpu.make_async_copy(b1_hbm, b1, wsems.at[5])
    c_w2 = pltpu.make_async_copy(w2_hbm, w2, wsems.at[6])

    x_copy(0).start()
    c_wk.start()
    for p in (1, 2, 3):
        x_copy(p).start()
    c_wq.start()
    c_wv.start()
    for p in range(4, NPAIR):
        x_copy(p).start()
    c_wo.start()
    c_b1.start()
    c_w1.start()
    c_w2.start()
    qz0[...] = jnp.zeros(qz0.shape, I32)
    qz1[...] = jnp.zeros(qz1.shape, I32)

    def prep_pieces(dst, load, hr, hc, transposed=False):
        def piece(r, c):
            def run():
                raw = [load(r, PR, c), load(r, PR, hc + c), load(hr + r, PR, c), load(hr + r, PR, hc + c)]
                if transposed:
                    raw[1], raw[2] = raw[2], raw[1]
                for i, t in enumerate(_st_b(*[t.astype(F32) for t in raw])):
                    t = raw[0] if i == 1 else raw[3] if i == 4 else t.astype(BF16)
                    dst[i, r // 2:(r + PR) // 2, c:c + 128] = _p32(t)
            return run
        return [piece(r, c) for r in range(0, hr, PR) for c in range(0, hc, 128)]

    def ref_loader(w):
        return lambda r, n, c: w[r:r + n, c:c + 128]

    def prep_transposed(dst, w):
        wt = w[...].T
        for t in prep_pieces(dst, lambda r, n, c: wt[r:r + n, c:c + 128], HD, HD, True):
            t()

    def qkv_dots(xn_top, xn_bot, row0):
        xc = [c.astype(BF16) for c in _st_a(xn_top[:, :HD], xn_top[:, HD:], xn_bot[:, :HD], xn_bot[:, HD:])]

        def k_part():
            c11, c12, c21, c22 = _st_c([_dot(xc[i], _u32(wkc[i])) for i in range(7)])
            for t, (cl, cr) in enumerate(((c11, c12), (c21, c22))):
                rows = pl.ds(pl.multiple_of((row0 + t * 128) // 2, 64), 64)
                for g, blk in enumerate((cl[:, :128], cl[:, 128:], cr[:, :128], cr[:, 128:])):
                    k4[g, rows, :] = _p32(blk.astype(BF16))

        def t_part(wc, dst, scale):
            def run():
                c11, c12, c21, c22 = _st_c([_dot_nt(_u32(wc[i]), xc[i]) for i in range(7)])
                for t, (cl, cr) in enumerate(((c11, c12), (c21, c22))):
                    for o, blk in enumerate((cl, cr)):
                        blk = blk if scale is None else blk * scale
                        dst[o * 128:(o + 1) * 128, half_rows(row0, t)] = _p32(blk.astype(BF16))
            return run

        return [k_part, t_part(wqc, qt, LOG2E * DH ** -0.5), t_part(wvc, vt, None)]

    def qkv_first():
        parts = {}

        def ln(p):
            xn = []
            for t in range(2):
                x = xin[half_rows(p * 256, t), :].astype(F32)
                xres[half_rows(p * 256, t), :] = x
                xn.append(_layernorm(x))
            parts[p] = qkv_dots(xn[0], xn[1], p * 256)

        x_copy(0).wait()
        ln(0)
        c_wk.wait()
        for t in prep_pieces(wkc, ref_loader(wk), HD, HD):
            t()
        x_copy(1).wait()
        parts[0][0]()
        ln(1)
        x_copy(2).wait()
        x_copy(3).wait()
        parts[1][0]()
        ln(2)
        ln(3)
        parts[2][0]()
        c_wq.wait()
        c_wv.wait()
        prep_transposed(wqc, wq)
        parts[3][0]()
        prep_transposed(wvc, wv)
        for p in (0, 1, 2):
            parts[p][1]()
        for p in (0, 1, 2):
            parts[p][2]()
        for p in range(4, NPAIR):
            x_copy(p).wait()
        for p in range(4, NPAIR):
            ln(p)
        parts[3][1]()
        parts[3][2]()
        for p in range(4, NPAIR):
            for t in parts[p]:
                t()

    def setq(i, qz):
        g, qb, h = _decode(i)
        hp = (h + 6) & 7
        qz[pl.ds(pl.multiple_of(hp * 8, 8), 8), :] = jnp.zeros((8, NQ), I32)
        qz[pl.ds(pl.multiple_of(h * 8, 8), 8), :] = qt[
            pl.ds(pl.multiple_of(g * 64 + h * 8, 8), 8), pl.ds(pl.multiple_of(qb * NQ, NQ), NQ)]

    def a_chunk(i, sref, qz, c, m8):
        g, qb, h = _decode(i)
        k = _u32(k4[g, pl.ds(c * CH // 2, CH // 2), :])
        s = _dot(k, _u32(qz[...]))
        sref[pl.ds(c * CH, CH), :] = s
        return jnp.maximum(m8, jnp.max(s.reshape(CH // 8, 8, NQ), axis=0))

    def b_chunk(i, sref, m, c, l8, acc, hist):
        g, qb, h = _decode(i)
        r0 = c * CH
        s = sref[pl.ds(r0, CH), :]
        mm = m
        if len(hist) >= LAG:
            mm = jnp.minimum(mm, jnp.maximum(mm, hist[-LAG][0:8]))
        p = jnp.exp2(s.reshape(CH // 8, 8, NQ) - mm[None]).reshape(CH, NQ)
        pb = p.astype(BF16)
        for j in reversed(range(CH // 8)):
            l8 = l8 + p[8 * j:8 * j + 8]
        v = _u32(vt[pl.ds(pl.multiple_of(g * 64 + h * 8, 8), 8), pl.ds(r0, CH)])
        d = _dot(v, pb)
        hist.append(d)
        return l8, acc + d

    def b_fin(i, l8, acc):
        g, qb, h = _decode(i)
        o = acc / jnp.sum(l8, axis=0, keepdims=True)
        ot[pl.ds(pl.multiple_of(g * 64 + h * 8, 8), 8), pl.ds(pl.multiple_of(qb * NQ, NQ), NQ)] = _p32(o.astype(BF16))

    def run_stream(ib, a_lo, a_hi, st, n_a, filler=None):
        hist = []
        nfill = -(-len(filler) // (a_hi - a_lo)) if filler else 0
        for a in range(a_lo, a_hi):
            if n_a is None or a < n_a:
                di, c = divmod(a, NCH)
                sref, qz = (s0, qz0) if di % 2 == 0 else (s1, qz1)
                if c == 0:
                    setq(ib + di, qz)
                    st.m8 = jnp.full((8, NQ), -jnp.inf, F32)
                st.m8 = a_chunk(ib + di, sref, qz, c, st.m8)
                if c == NCH - 1:
                    st.m_next = jnp.broadcast_to(jnp.max(st.m8, axis=0, keepdims=True), (8, NQ))
                    st.m8 = None
                for _ in range(nfill):
                    if filler:
                        filler.pop(0)()
            b = a - LAGC
            if b >= 0:
                di, c = divmod(b, NCH)
                if c == 0:
                    st.m = st.mq.pop(0)
                    st.l8 = jnp.zeros((8, NQ), F32)
                    st.acc = jnp.zeros((16, NQ), F32)
                st.l8, st.acc = b_chunk(ib + di, s0 if di % 2 == 0 else s1, st.m, c, st.l8, st.acc, hist)
                if c == NCH - 1:
                    b_fin(ib + di, st.l8, st.acc)
            if st.m8 is None and st.m_next is not None:
                st.mq.append(st.m_next)
                st.m_next = None

    def attention(first):
        per = UNROLL * NCH
        ntot = NITEMS * NCH
        nloop = (ntot - A0) // per
        st = _Stream()
        st.mq, st.m8, st.m_next = [], None, None
        st.m = st.l8 = st.acc = None
        filler = None
        if first:
            c_wo.wait()
            c_b1.wait()
            c_w1.wait()
            c_w2.wait()
            filler = prep_pieces(w1c, ref_loader(w1), HD, HF) + prep_pieces(w2c, ref_loader(w2), HF, HD)
        run_stream(0, 0, A0, st, None, filler)

        def pack(s):
            return tuple(s.mq), s.m8, s.m, s.l8, s.acc

        def unpack(carry):
            s = _Stream()
            s.mq, s.m8, s.m, s.l8, s.acc = list(carry[0]), *carry[1:]
            s.m_next = None
            return s

        def body(j, carry):
            s = unpack(carry)
            run_stream(j * UNROLL, A0, A0 + per, s, None)
            return pack(s)

        carry = lax.fori_loop(0, nloop, body, pack(st))
        n_a = ntot - nloop * per
        run_stream(nloop * UNROLL, A0, n_a + LAGC, unpack(carry), n_a)
        qz0[...] = jnp.zeros(qz0.shape, I32)
        qz1[...] = jnp.zeros(qz1.shape, I32)

    def post_tile(r, last):
        r0 = r * TM
        nj = HF // 128
        bias = b1[...].astype(F32).reshape(1, F)
        hv = [(p, t) for p in range(NP) for t in range(2)]
        a = {k: _dot_tn(_u32(ot[:, half_rows(r0 + k[0] * 256, k[1])]), wo[...]) for k in hv}
        x1 = {k: xres[half_rows(r0 + k[0] * 256, k[1]), :] + a[k] for k in hv}
        xn = {k: _layernorm(x1[k]) for k in hv}
        xc = [[c.astype(BF16) for c in _st_a(xn[p, 0][:, :HD], xn[p, 0][:, HD:], xn[p, 1][:, :HD], xn[p, 1][:, HD:])]
              for p in range(NP)]
        acc = [None] * NP
        hs = {}
        pending = []

        def f1(p, j):
            c0 = slice(j * 128, (j + 1) * 128)
            c1 = slice(HF + j * 128, HF + (j + 1) * 128)
            c11, c12, c21, c22 = _st_c([_dot(xc[p][i], _u32(w1c[i, :, c0])) for i in range(7)])
            hs[p, j] = (c11 + bias[:, c0], c12 + bias[:, c1], c21 + bias[:, c0], c22 + bias[:, c1])

        def f2(p, j):
            acts = [_mish(t) for t in hs.pop((p, j))]
            m = [_dot(t.astype(BF16), _u32(w2c[i, j * 64:(j + 1) * 64, :])) for i, t in enumerate(_st_a(*acts))]
            acc[p] = m if acc[p] is None else [x + y for x, y in zip(acc[p], m)]
            if j == nj - 1:
                c11, c12, c21, c22 = _st_c(acc[p])
                x2 = [x1[p, t] + jnp.concatenate(cc, axis=1) for t, cc in enumerate(((c11, c12), (c21, c22)))]
                for t in range(2):
                    rows = half_rows(r0 + p * 256, t)
                    if last:
                        obuf[rows, :] = x2[t].astype(BF16)
                        o_copy(r * NP + p, t).start()
                    else:
                        xres[rows, :] = x2[t]
                if not last:
                    pending.extend(qkv_dots(_layernorm(x2[0]), _layernorm(x2[1]), r0 + p * 256))

        tasks = [(p, j) for p in range(NP) for j in range(nj)]
        f1(*tasks[0])
        for n, t in enumerate(tasks):
            if n + 1 < len(tasks):
                f1(*tasks[n + 1])
            elif pending:
                pending.pop(0)()
            f2(*t)
        while pending:
            pending.pop(0)()

    qkv_first()
    for layer in range(N_LAYERS):
        attention(layer == 0)
        last = layer == N_LAYERS - 1
        lax.fori_loop(0, NT, lambda r, c, last=last: (post_tile(r, last), c)[1], 0)
    for p in range(NPAIR):
        for t in range(2):
            o_copy(p, t).wait()


@jax.jit
def pallas_interleave_layers__mha_block__dense_activation_mish__prompt_kernel(
    A_x: jax.Array,
    A_wqkv: jax.Array,
    A_wo: jax.Array,
    B_x: jax.Array,
    B_w1: jax.Array,
    B_b1: jax.Array,
    B_w2: jax.Array,
):
    del B_x
    vm = pltpu.VMEM
    any_spec = pl.BlockSpec(memory_space=pl.ANY)
    out = pl.pallas_call(
        _kernel,
        out_shape=jax.ShapeDtypeStruct((S, D), BF16),
        in_specs=[any_spec] * 6,
        out_specs=any_spec,
        scratch_shapes=[
            vm((S, D), BF16),
            vm((S, D), F32),
            vm((D, D), BF16),
            vm((D, D), BF16),
            vm((D, D), BF16),
            vm((D, D), BF16),
            vm((D, F), BF16),
            vm((F,), BF16),
            vm((F, D), BF16),
            vm((7, HD // 2, HD), I32),
            vm((7, HD // 2, HD), I32),
            vm((7, HD // 2, HD), I32),
            vm((7, HD // 2, HF), I32),
            vm((7, HF // 2, HD), I32),
            vm((4, S // 2, 128), I32),
            vm((D // 2, S), I32),
            vm((D // 2, S), I32),
            vm((D // 2, S), I32),
            vm((S, NQ), F32),
            vm((S, NQ), F32),
            vm((64, NQ), I32),
            vm((64, NQ), I32),
            vm((S, D), BF16),
            pltpu.SemaphoreType.DMA((NPAIR,)),
            pltpu.SemaphoreType.DMA((7,)),
            pltpu.SemaphoreType.DMA((2 * NPAIR,)),
        ],
        compiler_params=pltpu.CompilerParams(vmem_limit_bytes=100 * 1024 * 1024),
    )(A_x.reshape(S, D), A_wqkv, A_wo, B_w1, B_b1, B_w2)
    return out.reshape(1, S, D)
```
